```python
import os as _os
_os.environ.setdefault("JAX_PLATFORMS", "cpu")
import jax
import jax.numpy as jnp

def _softmax(x, axis=-1):
    return jax.nn.softmax(x, axis=axis)
def _gelu(x):
    return jax.nn.gelu(x, approximate=True)
def _silu(x):
    return jax.nn.silu(x)
def _sigmoid(x):
    return jax.nn.sigmoid(x)
def _layernorm(x, axis=-1, eps=1e-5):
    m = jnp.mean(x, axis=axis, keepdims=True)
    v = jnp.var(x, axis=axis, keepdims=True)
    return (x - m) / jnp.sqrt(v + eps)
def _scatter_add(tgt, idx, src, axis=0):
    return tgt.at[idx].add(src)
def _segment_sum(src, seg, n):
    return jax.ops.segment_sum(src, seg, n)
class _Rng:
    def __init__(self, key):
        self._k = key
    def _next(self):
        self._k, sub = jax.random.split(self._k)
        return sub
    def normal(self, shape):
        return jax.random.normal(self._next(), shape, dtype=jnp.bfloat16)
    def randint(self, lo, hi, shape):
        return jax.random.randint(self._next(), shape, lo, hi, dtype=jnp.int32)
    def uniform(self, shape, lo=0.0, hi=1.0):
        return jax.random.uniform(self._next(), shape, jnp.bfloat16, lo, hi)
    def permutation(self, n):
        return jax.random.permutation(self._next(), n)


kernel_name = 'gated_mix__linear_attn_block__glu_gated_swiglu__prompt'

def setup_inputs():
    _rng = _Rng(jax.random.key(int.from_bytes(__import__("os").urandom(4), "little")))
    _w = (lambda a: (lambda t: t.astype(jnp.bfloat16) if jnp.issubdtype(t.dtype, jnp.floating) else t)(jnp.asarray(a)))
    def _A_setup():
        B, S, D = 1, 2048, 1024
        return {
            "x": _w((lambda *s: _rng.normal(s) * 0.05)(B, S, D)),
            "wqkv": _w((lambda *s: _rng.normal(s) * 0.8)(D, 3 * D)),
            "wo": _w((lambda *s: _rng.normal(s) * 0.05)(D, D)),
        }
    _A_in = _A_setup()

    def _B_setup():
        B, S, D, F = 1, 2048, 1024, 3584
        return {
            "x": _w((lambda *s: _rng.normal(s) * 0.05)(B, S, D)),
            "w1": _w((lambda *s: _rng.normal(s) * 1.6)(D, F) * (2.0 / D) ** 0.5),
            "w3": _w((lambda *s: _rng.normal(s) * 1.6)(D, F) * (2.0 / D) ** 0.5),
            "w2": _w((lambda *s: _rng.normal(s) * 1.6)(F, D) * (2.0 / F) ** 0.5),
        }
    _B_in = _B_setup()

    return {
        "A_x": _A_in["x"],
        "A_wqkv": _A_in["wqkv"],
        "A_wo": _A_in["wo"],
        "B_x": _B_in["x"],
        "B_w1": _B_in["w1"],
        "B_w3": _B_in["w3"],
        "B_w2": _B_in["w2"],
        "gate_w": _w((lambda *s: _rng.normal(s) * 0.05)(1024) * 16.0),
    }

def reference(A_x, A_wqkv, A_wo, B_x, B_w1, B_w3, B_w2, gate_w):
    def _A_ref(x, wqkv, wo):
        B, S, D = x.shape
        H = 32; Dh = D // H
        qkv = (lambda x, *d: x.transpose(*d))((x @ wqkv).reshape(B, S, 3, H, Dh), 2, 0, 3, 1, 4)
        q, k, v = qkv[0], qkv[1], qkv[2]
        phi = lambda t: jnp.where(t > 0, t + 1, jnp.exp(t)) + 1e-6
        pq, pk = phi(q), phi(k)
        kv = jnp.einsum("bhsd,bhse->bhde", pk, v)
        z = jnp.einsum("bhsd->bhd", pk)
        num = jnp.einsum("bhqd,bhde->bhqe", pq, kv)
        den = jnp.einsum("bhqd,bhd->bhq", pq, z)[..., None] + 1e-6
        o = num / den
        return (lambda x, *d: x.transpose(*d))(o, 0, 2, 1, 3).reshape(B, S, D) @ wo

    def _B_ref(x, w1, w3, w2):
        gate = jnp.einsum("bsd,df->bsf", x, w1)
        up = jnp.einsum("bsd,df->bsf", x, w3)
        h = _silu(gate) * up
        out = jnp.einsum("bsf,fd->bsd", h, w2)
        return out

    x = A_x
    g = _sigmoid((x * gate_w).sum(-1, keepdims=True))
    a = _A_ref(x, A_wqkv, A_wo)
    b = _B_ref(x, B_w1, B_w3, B_w2)
    return g * a + (1 - g) * b
```

```python
import jax
import jax.numpy as jnp
import jax.experimental.pallas as pl
import jax.experimental.pallas.tpu as pltpu

S, D, F = 2048, 1024, 3584
DH = 32
CQ = 256
CF = 512
TM = 512
N_KV = D // CQ
N_Q = D // CQ
N_F = F // CF
N_STEPS = N_KV + N_Q + N_F
NSUB = CQ // 128
N_ROW = S // TM


def _phi(t):
    return jnp.where(t > 0, t + 1.0, jnp.exp(t)) + 1e-6


def _kernel(x_ref, wa_ref, wb_ref, wo_ref, w1_ref, w3_ref, w2_ref, gw_ref, out_ref,
            acc_ref, m_ref, zb_ref, g_ref, kv_ref, z_ref):
    step = pl.program_id(0)
    f32 = jnp.float32
    bf16 = jnp.bfloat16

    @pl.when(step == 0)
    def _():
        gw = gw_ref[...].astype(f32)

        def body(i, c):
            rows = pl.ds(pl.multiple_of(i * TM, TM), TM)
            xt = x_ref[rows, :].astype(f32)
            logit = jnp.sum(xt * gw, axis=-1, keepdims=True)
            g_ref[rows, :] = jax.nn.sigmoid(logit)
            return c
        jax.lax.fori_loop(0, N_ROW, body, 0)

    @pl.when(step < N_KV)
    def _():
        kv_ref[...] = jnp.zeros(kv_ref.shape, f32)
        z_ref[...] = jnp.zeros(z_ref.shape, f32)

        def body(i, c):
            rows = pl.ds(pl.multiple_of(i * TM, TM), TM)
            xt = x_ref[rows, :]
            k = jnp.dot(xt, wa_ref[...], preferred_element_type=f32)
            v = jnp.dot(xt, wb_ref[...], preferred_element_type=f32)
            pk = _phi(k)
            z_ref[...] += jnp.sum(pk, axis=0, keepdims=True)
            pkb = pk.astype(bf16)
            vb = v.astype(bf16)
            for j in range(NSUB):
                kv_ref[j] += jax.lax.dot_general(
                    pkb[:, j * 128:(j + 1) * 128], vb[:, j * 128:(j + 1) * 128],
                    (((0,), (0,)), ((), ())), preferred_element_type=f32)
            return c
        jax.lax.fori_loop(0, N_ROW, body, 0)

        r = jax.lax.broadcasted_iota(jnp.int32, (128, 128), 0) // DH
        cidx = jax.lax.broadcasted_iota(jnp.int32, (128, 128), 1) // DH
        mask = r == cidx
        for j in range(NSUB):
            off = pl.multiple_of(step * CQ + j * 128, 128)
            kvm = jnp.where(mask, kv_ref[j], 0.0).astype(bf16)
            m_ref[pl.ds(off, 128), :] = jnp.dot(
                kvm, wo_ref[pl.ds(off, 128), :], preferred_element_type=f32).astype(bf16)
            zrow = z_ref[:, j * 128:(j + 1) * 128]
            zcol = jnp.transpose(jnp.broadcast_to(zrow, (128, 128)))
            zb_ref[step * NSUB + j] = jnp.where(mask, zcol, 0.0).astype(bf16)

    @pl.when(jnp.logical_and(step >= N_KV, step < N_KV + N_Q))
    def _():
        c = step - N_KV

        def compute(i):
            rows = pl.ds(pl.multiple_of(i * TM, TM), TM)
            xt = x_ref[rows, :]
            q = jnp.dot(xt, wa_ref[...], preferred_element_type=f32)
            pq = _phi(q)
            pqb = pq.astype(bf16)
            g = g_ref[rows, :]
            parts = []
            for j in range(NSUB):
                den = jnp.dot(pqb[:, j * 128:(j + 1) * 128], zb_ref[c * NSUB + j],
                              preferred_element_type=f32) + 1e-6
                parts.append((pq[:, j * 128:(j + 1) * 128] * g / den).astype(bf16))
            r = jnp.concatenate(parts, axis=1)
            off = pl.multiple_of(c * CQ, CQ)
            return rows, jnp.dot(r, m_ref[pl.ds(off, CQ), :], preferred_element_type=f32)

        @pl.when(c == 0)
        def _():
            def body(i, cc):
                rows, contrib = compute(i)
                acc_ref[rows, :] = contrib
                return cc
            jax.lax.fori_loop(0, N_ROW, body, 0)

        @pl.when(c > 0)
        def _():
            def body(i, cc):
                rows, contrib = compute(i)
                acc_ref[rows, :] += contrib
                return cc
            jax.lax.fori_loop(0, N_ROW, body, 0)

    @pl.when(step >= N_KV + N_Q)
    def _():
        def compute(i):
            rows = pl.ds(pl.multiple_of(i * TM, TM), TM)
            xt = x_ref[rows, :]
            gate = jnp.dot(xt, w1_ref[...], preferred_element_type=f32)
            up = jnp.dot(xt, w3_ref[...], preferred_element_type=f32)
            omg = 1.0 - g_ref[rows, :]
            h = (gate * jax.nn.sigmoid(gate) * up * omg).astype(bf16)
            return rows, jnp.dot(h, w2_ref[...], preferred_element_type=f32)

        @pl.when(step < N_STEPS - 1)
        def _():
            def body(i, cc):
                rows, contrib = compute(i)
                acc_ref[rows, :] += contrib
                return cc
            jax.lax.fori_loop(0, N_ROW, body, 0)

        @pl.when(step == N_STEPS - 1)
        def _():
            def body(i, cc):
                rows, contrib = compute(i)
                out_ref[rows, :] = (acc_ref[rows, :] + contrib).astype(out_ref.dtype)
                return cc
            jax.lax.fori_loop(0, N_ROW, body, 0)


def _wa_map(s):
    return (0, jnp.where(s < N_KV, N_Q + s, jnp.minimum(s - N_KV, N_Q - 1)))


def _wb_map(s):
    return (0, 2 * N_Q + jnp.minimum(s, N_KV - 1))


def _f_idx(s):
    return jnp.maximum(s - (N_KV + N_Q), 0)


@jax.jit
def pallas_gated_mix__linear_attn_block__glu_gated_swiglu__prompt_kernel(
    A_x: jax.Array,
    A_wqkv: jax.Array,
    A_wo: jax.Array,
    B_x: jax.Array,
    B_w1: jax.Array,
    B_w3: jax.Array,
    B_w2: jax.Array,
    gate_w: jax.Array,
):
    x = A_x.reshape(S, D)
    gw = gate_w.reshape(1, D)
    one = pl.Buffered(1)
    out = pl.pallas_call(
        _kernel,
        grid=(N_STEPS,),
        in_specs=[
            pl.BlockSpec((S, D), lambda s: (0, 0), pipeline_mode=one),
            pl.BlockSpec((D, CQ), _wa_map),
            pl.BlockSpec((D, CQ), _wb_map),
            pl.BlockSpec((D, D), lambda s: (0, 0), pipeline_mode=one),
            pl.BlockSpec((D, CF), lambda s: (0, _f_idx(s))),
            pl.BlockSpec((D, CF), lambda s: (0, _f_idx(s))),
            pl.BlockSpec((CF, D), lambda s: (_f_idx(s), 0)),
            pl.BlockSpec((1, D), lambda s: (0, 0), pipeline_mode=one),
        ],
        out_specs=pl.BlockSpec((S, D), lambda s: (0, 0)),
        out_shape=jax.ShapeDtypeStruct((S, D), jnp.bfloat16),
        scratch_shapes=[
            pltpu.VMEM((S, D), jnp.float32),
            pltpu.VMEM((D, D), jnp.bfloat16),
            pltpu.VMEM((D // 128, 128, 128), jnp.bfloat16),
            pltpu.VMEM((S, 1), jnp.float32),
            pltpu.VMEM((NSUB, 128, 128), jnp.float32),
            pltpu.VMEM((1, CQ), jnp.float32),
        ],
        compiler_params=pltpu.CompilerParams(
            dimension_semantics=("arbitrary",),
            vmem_limit_bytes=100 * 1024 * 1024,
        ),
    )(x, A_wqkv, A_wqkv, A_wo, B_w1, B_w3, B_w2, gw)
    return out.reshape(1, S, D)
```

```python
import jax
import jax.numpy as jnp
import jax.experimental.pallas as pl
import jax.experimental.pallas.tpu as pltpu

S, D, F = 2048, 1024, 3584
DH = 32
CQ = 256
CF = 512
TX = 256
TB = 1024
TM = 512
OC = 256
N_C = D // CQ
N_F = F // CF
NSUB = CQ // 128
N_X = S // TX
N_B = S // TB
N_L = S // TM
assert N_F == 2 * N_C - 1
assert NSUB == N_B

SX = 0
SQ = SX + N_X
SK = SQ + N_C
SV = SK + N_C
SWO = SV + N_C
SW1 = SWO + N_C
SW3 = SW1 + N_F
SW2 = SW3 + N_F
SGW = SW2 + N_F
SOUT = SGW + 1
SOC = SOUT + N_L - 1
N_SEM = SOC + D // OC


def _phi(t):
    return jnp.where(t > 0, t + 1.0, jnp.exp(t)) + 1e-6


def _kernel(x_hbm, wqkv_hbm, wo_hbm, w1_hbm, w3_hbm, w2_hbm, gw_hbm, out_hbm,
            x_v, wq_v, wk_v, wv_v, wo_v, w1_v, w3_v, w2_v, gw_v, out_v,
            acc_ref, m_ref, zr_ref, g_ref, kv_ref, z_ref, pk_s, v_s, sems):
    f32 = jnp.float32
    bf16 = jnp.bfloat16

    def row_slice(i, tm):
        return pl.ds(pl.multiple_of(i * tm, tm), tm)

    def cp_x(i):
        return pltpu.make_async_copy(
            x_hbm.at[row_slice(i, TX)], x_v.at[row_slice(i, TX)], sems.at[SX + i])

    def cp_qkv(which, c):
        dst = (wq_v, wk_v, wv_v)[which]
        sem = (SQ, SK, SV)[which]
        col = pl.multiple_of(which * D + c * CQ, CQ)
        return pltpu.make_async_copy(wqkv_hbm.at[:, pl.ds(col, CQ)], dst.at[c], sems.at[sem + c])

    def cp_wo(c):
        rows = pl.ds(pl.multiple_of(c * CQ, CQ), CQ)
        return pltpu.make_async_copy(wo_hbm.at[rows], wo_v.at[rows], sems.at[SWO + c])

    def cp_w1(f):
        return pltpu.make_async_copy(
            w1_hbm.at[:, pl.ds(pl.multiple_of(f * CF, CF), CF)], w1_v.at[f], sems.at[SW1 + f])

    def cp_w3(f):
        return pltpu.make_async_copy(
            w3_hbm.at[:, pl.ds(pl.multiple_of(f * CF, CF), CF)], w3_v.at[f], sems.at[SW3 + f])

    def cp_w2(f):
        return pltpu.make_async_copy(
            w2_hbm.at[pl.ds(pl.multiple_of(f * CF, CF), CF)], w2_v.at[f], sems.at[SW2 + f])

    def cp_gw():
        return pltpu.make_async_copy(gw_hbm, gw_v, sems.at[SGW])

    def cp_out(i):
        return pltpu.make_async_copy(
            out_v.at[row_slice(i, TM)], out_hbm.at[row_slice(i, TM)], sems.at[SOUT + i])

    def cp_out_cols(b):
        rows = pl.ds(S - TM, TM)
        cols = pl.ds(b * OC, OC)
        return pltpu.make_async_copy(
            out_v.at[rows, cols], out_hbm.at[rows, cols], sems.at[SOC + b])

    def start_kv(c):
        cp_qkv(1, c).start()
        cp_qkv(2, c).start()
        cp_wo(c).start()

    def wait_kv(c):
        cp_qkv(1, c).wait()
        cp_qkv(2, c).wait()

    def start_ffn(f):
        cp_w1(f).start()
        cp_w3(f).start()
        cp_w2(f).start()

    def wait_ffn(f):
        cp_w1(f).wait()
        cp_w3(f).wait()
        cp_w2(f).wait()

    def kv_accumulate(slot, pkb, vb):
        for j in range(NSUB):
            kv_ref[slot, j] += jax.lax.dot_general(
                pkb[:, j * 128:(j + 1) * 128], vb[:, j * 128:(j + 1) * 128],
                (((0,), (0,)), ((), ())), preferred_element_type=f32)

    def kv_project(c, i, tm):
        slot = c % 2
        xt = x_v[row_slice(i, tm), :]
        k = jnp.dot(xt, wk_v[c], preferred_element_type=f32)
        v = jnp.dot(xt, wv_v[c], preferred_element_type=f32)
        pk = _phi(k)
        z_ref[slot] += jnp.sum(pk, axis=0, keepdims=True)
        return pk.astype(bf16), v.astype(bf16)

    def kv_unit(c, i, tm):
        pkb, vb = kv_project(c, i, tm)
        kv_accumulate(c % 2, pkb, vb)

    def kv_init(c):
        slot = c % 2
        kv_ref[slot] = jnp.zeros(kv_ref.shape[1:], f32)
        z_ref[slot] = jnp.zeros(z_ref.shape[1:], f32)

    def kv_tail(c, j):
        slot = c % 2
        r = jax.lax.broadcasted_iota(jnp.int32, (128, 128), 0) // DH
        cidx = jax.lax.broadcasted_iota(jnp.int32, (128, 128), 1) // DH
        mask = r == cidx
        off = pl.multiple_of(c * CQ + j * 128, 128)
        kvm = jnp.where(mask, kv_ref[slot, j], 0.0).astype(bf16)
        m_ref[pl.ds(off, 128), :] = jnp.dot(
            kvm, wo_v[pl.ds(off, 128), :], preferred_element_type=f32).astype(bf16)
        zr_ref[c * NSUB + j] = z_ref[slot, :, pl.ds(pl.multiple_of(j * 128, 128), 128)]

    def group_sum(t):
        lane = jax.lax.broadcasted_iota(jnp.int32, t.shape, 1)
        sh = DH // 2
        while sh >= 1:
            up = pltpu.roll(t, sh, 1)
            dn = pltpu.roll(t, 128 - sh, 1)
            t = t + jnp.where((lane & sh) != 0, up, dn)
            sh //= 2
        return t

    def q_lhs(c, i, tm):
        rows = row_slice(i, tm)
        xt = x_v[rows, :]
        q = jnp.dot(xt, wq_v[c], preferred_element_type=f32)
        pq = _phi(q)
        g = g_ref[rows, :]
        parts = []
        for j in range(NSUB):
            pj = pq[:, j * 128:(j + 1) * 128]
            den = group_sum(pj * zr_ref[c * NSUB + j]) + 1e-6
            parts.append((pj * g / den).astype(bf16))
        return jnp.concatenate(parts, axis=1)

    def q_unit(c, i, tm):
        off = pl.multiple_of(c * CQ, CQ)
        return jnp.dot(q_lhs(c, i, tm), m_ref[pl.ds(off, CQ), :], preferred_element_type=f32)

    def f_lhs(f, i, tm, g=None):
        rows = row_slice(i, tm)
        xt = x_v[rows, :]
        gate = jnp.dot(xt, w1_v[f], preferred_element_type=f32)
        up = jnp.dot(xt, w3_v[f], preferred_element_type=f32)
        if g is None:
            g = g_ref[rows, :]
        return (gate * jax.nn.sigmoid(gate) * up * (1.0 - g)).astype(bf16)

    def f_unit(f, i, tm, g=None):
        return jnp.dot(f_lhs(f, i, tm, g), w2_v[f], preferred_element_type=f32)

    cp_x(0).start()
    cp_qkv(1, 0).start()
    cp_qkv(2, 0).start()
    cp_gw().start()
    kv_init(0)
    cp_x(0).wait()
    cp_qkv(1, 0).wait()
    for i in range(1, N_X):
        cp_x(i).start()
    cp_wo(0).start()
    start_kv(1)
    start_ffn(0)

    def s0_tile(i, first):
        cur = i % 2
        rows = row_slice(i, TX)
        xt = x_v[rows, :]
        k = jnp.dot(xt, wk_v[0], preferred_element_type=f32)
        if first:
            cp_qkv(2, 0).wait()
            cp_gw().wait()
        else:
            prev = (i + 1) % 2
            kv_accumulate(0, pk_s[prev], v_s[prev])
        gw = gw_v[...].astype(f32)
        g_ref[rows, :] = jax.nn.sigmoid(
            jnp.sum(xt.astype(f32) * gw, axis=-1, keepdims=True))
        v = jnp.dot(xt, wv_v[0], preferred_element_type=f32)
        pk = _phi(k)
        z_ref[0] += jnp.sum(pk, axis=0, keepdims=True)
        pk_s[cur] = pk.astype(bf16)
        v_s[cur] = v.astype(bf16)

    s0_tile(0, True)

    def body0(i, cc):
        cp_x(i).wait()
        s0_tile(i, False)
        return cc
    jax.lax.fori_loop(1, N_X, body0, 0)
    kv_accumulate(0, pk_s[(N_X - 1) % 2], v_s[(N_X - 1) % 2])

    start_kv(2)
    start_ffn(1)
    wait_kv(1)
    wait_ffn(0)
    cp_wo(0).wait()
    kv_init(1)

    def body1(i, cc):
        kv_tail(0, i)
        kv_unit(1, i, TB)
        acc_ref[row_slice(i, TB), :] = f_unit(0, i, TB)
        return cc
    jax.lax.fori_loop(0, N_B, body1, 0)

    def kvf_stage(c, carry):
        @pl.when(c + 1 < N_C)
        def _():
            start_kv(c + 1)

        @pl.when(c + 1 == N_C)
        def _():
            cp_qkv(0, 0).start()
        start_ffn(c)
        wait_kv(c)
        wait_ffn(c - 1)
        cp_wo(c - 1).wait()
        kv_init(c)

        def body(i, cc):
            kv_tail(c - 1, i)
            kv_unit(c, i, TB)
            acc_ref[row_slice(i, TB), :] += f_unit(c - 1, i, TB)
            return cc
        jax.lax.fori_loop(0, N_B, body, 0)

        @pl.when(c == N_C - 1)
        def _():
            cp_wo(N_C - 1).wait()
            for j in range(NSUB):
                kv_tail(N_C - 1, j)
        return carry
    jax.lax.fori_loop(2, N_C, kvf_stage, 0)

    def qf_stage(c, carry):
        f = N_C - 1 + c
        cp_qkv(0, c + 1).start()
        start_ffn(f + 1)
        cp_qkv(0, c).wait()
        wait_ffn(f)

        def body(i, cc):
            acc_ref[row_slice(i, TB), :] += q_unit(c, i, TB) + f_unit(f, i, TB)
            return cc
        jax.lax.fori_loop(0, N_B, body, 0)
        return carry
    jax.lax.fori_loop(0, N_C - 1, qf_stage, 0)

    cp_qkv(0, N_C - 1).wait()
    wait_ffn(N_F - 1)

    def last_body(i, cc):
        rows = row_slice(i, TM)
        tot = acc_ref[rows, :] + (q_unit(N_C - 1, i, TM) + f_unit(N_F - 1, i, TM))
        out_v[rows, :] = tot.astype(out_v.dtype)
        cp_out(i).start()
        return cc
    jax.lax.fori_loop(0, N_L - 1, last_body, 0)

    rows = pl.ds(S - TM, TM)
    r = q_lhs(N_C - 1, N_L - 1, TM)
    h = f_lhs(N_F - 1, N_L - 1, TM)
    for b in range(D // OC):
        cols = pl.ds(b * OC, OC)
        tot = acc_ref[rows, cols] + (
            jnp.dot(r, m_ref[pl.ds(D - CQ, CQ), cols], preferred_element_type=f32)
            + jnp.dot(h, w2_v[N_F - 1, :, cols], preferred_element_type=f32))
        out_v[rows, cols] = tot.astype(out_v.dtype)
        cp_out_cols(b).start()

    for i in range(N_L - 1):
        cp_out(i).wait()
    for b in range(D // OC):
        cp_out_cols(b).wait()


@jax.jit
def pallas_gated_mix__linear_attn_block__glu_gated_swiglu__prompt_kernel(
    A_x: jax.Array,
    A_wqkv: jax.Array,
    A_wo: jax.Array,
    B_x: jax.Array,
    B_w1: jax.Array,
    B_w3: jax.Array,
    B_w2: jax.Array,
    gate_w: jax.Array,
):
    x = A_x.reshape(S, D)
    gw = gate_w.reshape(1, D)
    bf16 = jnp.bfloat16
    any_spec = pl.BlockSpec(memory_space=pl.ANY)
    out = pl.pallas_call(
        _kernel,
        in_specs=[any_spec] * 7,
        out_specs=any_spec,
        out_shape=jax.ShapeDtypeStruct((S, D), bf16),
        scratch_shapes=[
            pltpu.VMEM((S, D), bf16),
            pltpu.VMEM((N_C, D, CQ), bf16),
            pltpu.VMEM((N_C, D, CQ), bf16),
            pltpu.VMEM((N_C, D, CQ), bf16),
            pltpu.VMEM((D, D), bf16),
            pltpu.VMEM((N_F, D, CF), bf16),
            pltpu.VMEM((N_F, D, CF), bf16),
            pltpu.VMEM((N_F, CF, D), bf16),
            pltpu.VMEM((1, D), bf16),
            pltpu.VMEM((S, D), bf16),
            pltpu.VMEM((S, D), jnp.float32),
            pltpu.VMEM((D, D), bf16),
            pltpu.VMEM((D // 128, 1, 128), jnp.float32),
            pltpu.VMEM((S, 1), jnp.float32),
            pltpu.VMEM((2, NSUB, 128, 128), jnp.float32),
            pltpu.VMEM((2, 1, CQ), jnp.float32),
            pltpu.VMEM((2, TX, CQ), bf16),
            pltpu.VMEM((2, TX, CQ), bf16),
            pltpu.SemaphoreType.DMA((N_SEM,)),
        ],
        compiler_params=pltpu.CompilerParams(
            vmem_limit_bytes=100 * 1024 * 1024,
        ),
    )(x, A_wqkv, A_wo, B_w1, B_w3, B_w2, gw)
    return out.reshape(1, S, D)
```

```python
import jax
import jax.numpy as jnp
import jax.experimental.pallas as pl
import jax.experimental.pallas.tpu as pltpu

S, D, F = 2048, 1024, 3584
DH = 32
CQ = 256
CF = 512
TX = 256
TB = 1024
TM = 512
OC = 256
N_C = D // CQ
N_F = F // CF
NSUB = CQ // 128
N_X = S // TX
N_B = S // TB
N_L = S // TM
assert N_F == 2 * N_C - 1
assert NSUB == N_B

SX = 0
SQ = SX + N_X
SK = SQ + N_C
SV = SK + N_C
SWO = SV + N_C
SW1 = SWO + N_C
SW3 = SW1 + N_F
SW2 = SW3 + N_F
SGW = SW2 + N_F
SOUT = SGW + 1
SOC = SOUT + N_L - 1
N_SEM = SOC + D // OC


def _phi(t):
    return jnp.where(t > 0, t + 1.0, jnp.exp(t)) + 1e-6


def _kernel(x_hbm, wqkv_hbm, wo_hbm, w1_hbm, w3_hbm, w2_hbm, gw_hbm, out_hbm,
            x_v, wq_v, wk_v, wv_v, wo_v, w1_v, w3_v, w2_v, gw_v, out_v,
            acc_ref, m_ref, g_ref, kv_ref, z_ref, pk_s, v_s, sems):
    f32 = jnp.float32
    bf16 = jnp.bfloat16

    def row_slice(i, tm):
        return pl.ds(pl.multiple_of(i * tm, tm), tm)

    def cp_x(i):
        return pltpu.make_async_copy(
            x_hbm.at[row_slice(i, TX)], x_v.at[row_slice(i, TX)], sems.at[SX + i])

    def cp_qkv(which, c):
        dst = (wq_v, wk_v, wv_v)[which]
        sem = (SQ, SK, SV)[which]
        col = pl.multiple_of(which * D + c * CQ, CQ)
        return pltpu.make_async_copy(wqkv_hbm.at[:, pl.ds(col, CQ)], dst.at[c], sems.at[sem + c])

    def cp_wo(c):
        rows = pl.ds(pl.multiple_of(c * CQ, CQ), CQ)
        return pltpu.make_async_copy(wo_hbm.at[rows], wo_v.at[rows], sems.at[SWO + c])

    def cp_w1(f):
        return pltpu.make_async_copy(
            w1_hbm.at[:, pl.ds(pl.multiple_of(f * CF, CF), CF)], w1_v.at[f], sems.at[SW1 + f])

    def cp_w3(f):
        return pltpu.make_async_copy(
            w3_hbm.at[:, pl.ds(pl.multiple_of(f * CF, CF), CF)], w3_v.at[f], sems.at[SW3 + f])

    def cp_w2(f):
        return pltpu.make_async_copy(
            w2_hbm.at[pl.ds(pl.multiple_of(f * CF, CF), CF)], w2_v.at[f], sems.at[SW2 + f])

    def cp_gw():
        return pltpu.make_async_copy(gw_hbm, gw_v, sems.at[SGW])

    def cp_out(i):
        return pltpu.make_async_copy(
            out_v.at[row_slice(i, TM)], out_hbm.at[row_slice(i, TM)], sems.at[SOUT + i])

    def cp_out_cols(b):
        rows = pl.ds(S - TM, TM)
        cols = pl.ds(b * OC, OC)
        return pltpu.make_async_copy(
            out_v.at[rows, cols], out_hbm.at[rows, cols], sems.at[SOC + b])

    def wait_kv(c):
        cp_qkv(1, c).wait()
        cp_qkv(2, c).wait()

    def start_ffn(f):
        cp_w1(f).start()
        cp_w3(f).start()
        cp_w2(f).start()

    def wait_ffn(f):
        cp_w1(f).wait()
        cp_w3(f).wait()
        cp_w2(f).wait()

    def kv_accumulate(slot, pkb, vb):
        for j in range(NSUB):
            kv_ref[slot, j] += jax.lax.dot_general(
                pkb[:, j * 128:(j + 1) * 128], vb[:, j * 128:(j + 1) * 128],
                (((0,), (0,)), ((), ())), preferred_element_type=f32)

    def kv_project(c, i, tm):
        xt = x_v[row_slice(i, tm), :]
        k = jnp.dot(xt, wk_v[c], preferred_element_type=f32)
        v = jnp.dot(xt, wv_v[c], preferred_element_type=f32)
        pk = _phi(k)
        z_ref[c] += jnp.sum(pk, axis=0, keepdims=True)
        return pk.astype(bf16), v.astype(bf16)

    def kv_unit(c, i, tm):
        pkb, vb = kv_project(c, i, tm)
        kv_accumulate(c, pkb, vb)

    def kv_init(c):
        kv_ref[c] = jnp.zeros(kv_ref.shape[1:], f32)
        z_ref[c] = jnp.zeros(z_ref.shape[1:], f32)

    def kv_tail(c, j):
        r = jax.lax.broadcasted_iota(jnp.int32, (128, 128), 0) // DH
        cidx = jax.lax.broadcasted_iota(jnp.int32, (128, 128), 1) // DH
        mask = r == cidx
        off = pl.multiple_of(c * CQ + j * 128, 128)
        kvm = jnp.where(mask, kv_ref[c, j], 0.0).astype(bf16)
        m_ref[pl.ds(off, 128), :] = jnp.dot(
            kvm, wo_v[pl.ds(off, 128), :], preferred_element_type=f32).astype(bf16)

    def group_sum(t):
        lane = jax.lax.broadcasted_iota(jnp.int32, t.shape, 1)
        sh = DH // 2
        while sh >= 1:
            up = pltpu.roll(t, sh, 1)
            dn = pltpu.roll(t, 128 - sh, 1)
            t = t + jnp.where((lane & sh) != 0, up, dn)
            sh //= 2
        return t

    def q_lhs(c, i, tm):
        rows = row_slice(i, tm)
        xt = x_v[rows, :]
        q = jnp.dot(xt, wq_v[c], preferred_element_type=f32)
        pq = _phi(q)
        g = g_ref[rows, :]
        parts = []
        for j in range(NSUB):
            pj = pq[:, j * 128:(j + 1) * 128]
            den = group_sum(pj * z_ref[c, :, j * 128:(j + 1) * 128]) + 1e-6
            parts.append((pj * g / den).astype(bf16))
        return jnp.concatenate(parts, axis=1)

    def q_unit(c, i, tm):
        off = pl.multiple_of(c * CQ, CQ)
        return jnp.dot(q_lhs(c, i, tm), m_ref[pl.ds(off, CQ), :], preferred_element_type=f32)

    def f_lhs(f, i, tm):
        rows = row_slice(i, tm)
        xt = x_v[rows, :]
        gate = jnp.dot(xt, w1_v[f], preferred_element_type=f32)
        up = jnp.dot(xt, w3_v[f], preferred_element_type=f32)
        g = g_ref[rows, :]
        return (gate * jax.nn.sigmoid(gate) * up * (1.0 - g)).astype(bf16)

    def f_unit(f, i, tm):
        return jnp.dot(f_lhs(f, i, tm), w2_v[f], preferred_element_type=f32)

    cp_x(0).start()
    cp_qkv(1, 0).start()
    cp_qkv(2, 0).start()
    cp_gw().start()
    for i in range(1, N_X):
        cp_x(i).start()
    for c in range(1, N_C):
        cp_qkv(1, c).start()
        cp_qkv(2, c).start()
        start_ffn(c - 1)
        cp_wo(c - 1).start()
    cp_wo(N_C - 1).start()
    for c in range(N_C):
        cp_qkv(0, c).start()
        start_ffn(N_C - 1 + c)
    kv_init(0)
    cp_x(0).wait()
    cp_qkv(1, 0).wait()

    def s0_tile(i, first):
        cur = i % 2
        rows = row_slice(i, TX)
        xt = x_v[rows, :]
        k = jnp.dot(xt, wk_v[0], preferred_element_type=f32)
        if first:
            cp_qkv(2, 0).wait()
            cp_gw().wait()
        else:
            prev = (i + 1) % 2
            kv_accumulate(0, pk_s[prev], v_s[prev])
        gw = gw_v[...].astype(f32).reshape(1, D)
        g_ref[rows, :] = jax.nn.sigmoid(
            jnp.sum(xt.astype(f32) * gw, axis=-1, keepdims=True))
        v = jnp.dot(xt, wv_v[0], preferred_element_type=f32)
        pk = _phi(k)
        z_ref[0] += jnp.sum(pk, axis=0, keepdims=True)
        pk_s[cur] = pk.astype(bf16)
        v_s[cur] = v.astype(bf16)

    s0_tile(0, True)

    def body0(i, cc):
        cp_x(i).wait()
        s0_tile(i, False)
        return cc
    jax.lax.fori_loop(1, N_X, body0, 0)
    kv_accumulate(0, pk_s[(N_X - 1) % 2], v_s[(N_X - 1) % 2])

    wait_kv(1)
    wait_ffn(0)
    kv_init(1)

    def body1(i, cc):
        kv_unit(1, i, TB)
        acc_ref[row_slice(i, TB), :] = f_unit(0, i, TB)
        return cc
    jax.lax.fori_loop(0, N_B, body1, 0)

    def kvf_stage(c, carry):
        wait_kv(c)
        wait_ffn(c - 1)
        cp_wo(c - 2).wait()
        kv_init(c)

        def body(i, cc):
            kv_tail(c - 2, i)
            kv_unit(c, i, TB)
            acc_ref[row_slice(i, TB), :] += f_unit(c - 1, i, TB)
            return cc
        jax.lax.fori_loop(0, N_B, body, 0)
        return carry
    jax.lax.fori_loop(2, N_C, kvf_stage, 0)

    def qf_stage(c, carry):
        f = N_C - 1 + c
        cp_qkv(0, c).wait()
        wait_ffn(f)

        @pl.when(c + 2 < N_C)
        def _():
            cp_wo(c + 2).wait()

        def body(i, cc):
            kv_tail(jnp.minimum(c + 2, N_C - 1), i)
            acc_ref[row_slice(i, TB), :] += q_unit(c, i, TB) + f_unit(f, i, TB)
            return cc
        jax.lax.fori_loop(0, N_B, body, 0)
        return carry
    jax.lax.fori_loop(0, N_C - 1, qf_stage, 0)

    cp_qkv(0, N_C - 1).wait()
    wait_ffn(N_F - 1)

    def last_body(i, cc):
        rows = row_slice(i, TM)
        tot = acc_ref[rows, :] + (q_unit(N_C - 1, i, TM) + f_unit(N_F - 1, i, TM))
        out_v[rows, :] = tot.astype(out_v.dtype)
        cp_out(i).start()
        return cc
    jax.lax.fori_loop(0, N_L - 1, last_body, 0)

    rows = pl.ds(S - TM, TM)
    r = q_lhs(N_C - 1, N_L - 1, TM)
    h = f_lhs(N_F - 1, N_L - 1, TM)
    for b in range(D // OC):
        cols = pl.ds(b * OC, OC)
        tot = acc_ref[rows, cols] + (
            jnp.dot(r, m_ref[pl.ds(D - CQ, CQ), cols], preferred_element_type=f32)
            + jnp.dot(h, w2_v[N_F - 1, :, cols], preferred_element_type=f32))
        out_v[rows, cols] = tot.astype(out_v.dtype)
        cp_out_cols(b).start()

    for i in range(N_L - 1):
        cp_out(i).wait()
    for b in range(D // OC):
        cp_out_cols(b).wait()


@jax.jit
def pallas_gated_mix__linear_attn_block__glu_gated_swiglu__prompt_kernel(
    A_x: jax.Array,
    A_wqkv: jax.Array,
    A_wo: jax.Array,
    B_x: jax.Array,
    B_w1: jax.Array,
    B_w3: jax.Array,
    B_w2: jax.Array,
    gate_w: jax.Array,
):
    x = A_x.reshape(S, D)
    bf16 = jnp.bfloat16
    any_spec = pl.BlockSpec(memory_space=pl.ANY)
    out = pl.pallas_call(
        _kernel,
        in_specs=[any_spec] * 7,
        out_specs=any_spec,
        out_shape=jax.ShapeDtypeStruct((S, D), bf16),
        scratch_shapes=[
            pltpu.VMEM((S, D), bf16),
            pltpu.VMEM((N_C, D, CQ), bf16),
            pltpu.VMEM((N_C, D, CQ), bf16),
            pltpu.VMEM((N_C, D, CQ), bf16),
            pltpu.VMEM((D, D), bf16),
            pltpu.VMEM((N_F, D, CF), bf16),
            pltpu.VMEM((N_F, D, CF), bf16),
            pltpu.VMEM((N_F, CF, D), bf16),
            pltpu.VMEM((D,), bf16),
            pltpu.VMEM((S, D), bf16),
            pltpu.VMEM((S, D), jnp.float32),
            pltpu.VMEM((D, D), bf16),
            pltpu.VMEM((S, 1), jnp.float32),
            pltpu.VMEM((N_C, NSUB, 128, 128), jnp.float32),
            pltpu.VMEM((N_C, 1, CQ), jnp.float32),
            pltpu.VMEM((2, TX, CQ), bf16),
            pltpu.VMEM((2, TX, CQ), bf16),
            pltpu.SemaphoreType.DMA((N_SEM,)),
        ],
        compiler_params=pltpu.CompilerParams(
            vmem_limit_bytes=100 * 1024 * 1024,
        ),
    )(x, A_wqkv, A_wo, B_w1, B_w3, B_w2, gate_w)
    return out.reshape(1, S, D)
```
